```python
import os as _os
_os.environ.setdefault("JAX_PLATFORMS", "cpu")
import jax
import jax.numpy as jnp

def _softmax(x, axis=-1):
    return jax.nn.softmax(x, axis=axis)
def _gelu(x):
    return jax.nn.gelu(x, approximate=True)
def _silu(x):
    return jax.nn.silu(x)
def _sigmoid(x):
    return jax.nn.sigmoid(x)
def _layernorm(x, axis=-1, eps=1e-5):
    m = jnp.mean(x, axis=axis, keepdims=True)
    v = jnp.var(x, axis=axis, keepdims=True)
    return (x - m) / jnp.sqrt(v + eps)
def _scatter_add(tgt, idx, src, axis=0):
    return tgt.at[idx].add(src)
def _segment_sum(src, seg, n):
    return jax.ops.segment_sum(src, seg, n)
class _Rng:
    def __init__(self, key):
        self._k = key
    def _next(self):
        self._k, sub = jax.random.split(self._k)
        return sub
    def normal(self, shape):
        return jax.random.normal(self._next(), shape, dtype=jnp.bfloat16)
    def randint(self, lo, hi, shape):
        return jax.random.randint(self._next(), shape, lo, hi, dtype=jnp.int32)
    def uniform(self, shape, lo=0.0, hi=1.0):
        return jax.random.uniform(self._next(), shape, jnp.bfloat16, lo, hi)
    def permutation(self, n):
        return jax.random.permutation(self._next(), n)


kernel_name = 'sequential_preLN__ssm_conv_h3__mixer_s_mlp__prompt'

def setup_inputs():
    _rng = _Rng(jax.random.key(int.from_bytes(__import__("os").urandom(4), "little")))
    _w = (lambda a: (lambda t: t.astype(jnp.bfloat16) if jnp.issubdtype(t.dtype, jnp.floating) else t)(jnp.asarray(a)))
    def _A_setup():
        B, S, D = 1, 2048, 640
        ks = 4
        return {
            "q": _w((lambda *s: _rng.normal(s) * 0.05)(B, S, D)),
            "k": _w((lambda *s: _rng.normal(s) * 0.05)(B, S, D)),
            "v": _w((lambda *s: _rng.normal(s) * 0.05)(B, S, D)),
            "shift_k": _w((lambda *s: _rng.normal(s) * 0.05)(D, ks) * 0.5),
            "ssm_k": _w((lambda *s: _rng.normal(s) * 0.05)(D, S) * (1.0 / S ** 0.5)),
            "ssm_D": _w((lambda *s: _rng.normal(s) * 0.05)(D)),
        }
    _A_in = _A_setup()

    def _B_setup():
        B, S, D, F = 1, 2048, 640, 1728
        return {
            "x":  _w((lambda *s: _rng.normal(s) * 0.05)(B, S, D)),
            "w1": _w((lambda *s: _rng.normal(s) * 0.8)(D, D) * (D ** -0.5)),
            "w2": _w((lambda *s: _rng.normal(s) * 0.8)(D, D) * (D ** -0.5)),
            "w3": _w((lambda *s: _rng.normal(s) * 0.8)(D, F) * (D ** -0.5)),
            "w4": _w((lambda *s: _rng.normal(s) * 0.8)(F, D) * (F ** -0.5)),
        }
    _B_in = _B_setup()

    return {
        "A_q": _A_in["q"],
        "A_k": _A_in["k"],
        "A_v": _A_in["v"],
        "A_shift_k": _A_in["shift_k"],
        "A_ssm_k": _A_in["ssm_k"],
        "A_ssm_D": _A_in["ssm_D"],
        "B_x": _B_in["x"],
        "B_w1": _B_in["w1"],
        "B_w2": _B_in["w2"],
        "B_w3": _B_in["w3"],
        "B_w4": _B_in["w4"],
    }

def reference(A_q, A_k, A_v, A_shift_k, A_ssm_k, A_ssm_D, B_x, B_w1, B_w2, B_w3, B_w4):
    def _A_ref(q, k, v, shift_k, ssm_k, ssm_D):
        B, S, D = q.shape
        ks = shift_k.shape[-1]
        k_pad = jnp.pad(k, ((0, 0), (ks - 1, 0), (0, 0)))
        k_shift = jnp.zeros_like(k)
        for t in range(ks):
            k_shift = k_shift + k_pad[:, t:t + S, :] * shift_k[:, ks - 1 - t][None, None, :]
        kv = k_shift * v
        L = 2 * S
        kv_pad = jnp.pad(kv, ((0, 0), (0, S), (0, 0)))
        kf_pad = jnp.pad(ssm_k, ((0, 0), (0, S)))
        kv_f = (lambda x, axes=(-2,-1): jnp.fft.rfft2(x.astype(jnp.float32), axes=axes))(kv_pad[:, None, :, :], axes=(1, 2))
        kf_f = (lambda x, axes=(-2,-1): jnp.fft.rfft2(x.astype(jnp.float32), axes=axes))(kf_pad[:, None, :], axes=(1, 2))
        kf_f = (lambda x, *d: x.transpose(*d))(kf_f, 1, 2, 0)
        y_f = kv_f * kf_f[None, :, :, :]
        y = (lambda x, s, axes=(-2,-1): jnp.fft.irfft2(x, s=s, axes=axes).astype(jnp.bfloat16))(y_f, (1, L), axes=(1, 2))[:, 0, :S, :]
        y = y + kv * ssm_D[None, None, :]
        return q * y

    def _B_ref(x, w1, w2, w3, w4):
        B, S, D = x.shape
        h = _gelu(_layernorm(x, axis=-1) @ w1)
        c = D // 4
        g0 = jnp.pad(h[:, :, 0*c:1*c], ((0, 0), (1, 0), (0, 0)))[:, :S, :]
        g1 = jnp.pad(h[:, :, 1*c:2*c], ((0, 0), (0, 1), (0, 0)))[:, 1:, :]
        g2 = jnp.pad(h[:, :, 2*c:3*c], ((0, 0), (2, 0), (0, 0)))[:, :S, :]
        g3 = jnp.pad(h[:, :, 3*c:   ], ((0, 0), (0, 2), (0, 0)))[:, 2:, :]
        hs = jnp.concatenate([g0, g1, g2, g3], axis=-1) @ w2
        x1 = x + hs
        h2 = _gelu(_layernorm(x1, axis=-1) @ w3) @ w4
        return x1 + h2

    x = A_q
    h = x + _A_ref(_layernorm(x, axis=-1), A_k, A_v, A_shift_k, A_ssm_k, A_ssm_D)
    h2 = h + _B_ref(_layernorm(h, axis=-1), B_w1, B_w2, B_w3, B_w4)
    return h2
```

```python
import numpy as np
import jax
import jax.numpy as jnp
import jax.experimental.pallas as pl
import jax.experimental.pallas.tpu as pltpu

S, D, FF = 2048, 640, 1728
C = 128
NB = S // C
T = 256
NT = S // T
SUB = T // C
GRP = D // 4
EPS = 1e-5
F32 = jnp.float32
BF16 = jnp.bfloat16


def _dft_constants():
    f = np.arange(C, dtype=np.float64)
    theta = np.pi * (2.0 * f + 1.0) / (2.0 * C)
    r = np.arange(C, dtype=np.float64)
    ang = theta[:, None] * r[None, :]
    fw = np.concatenate([np.cos(ang), -np.sin(ang)], axis=0)
    n = np.arange(2 * C, dtype=np.float64)
    angn = n[:, None] * theta[None, :]
    gi = np.concatenate([np.cos(angn), -np.sin(angn)], axis=1) / C
    return fw.astype(np.float32), gi.astype(np.float32)


def _ln(x):
    m = jnp.mean(x, axis=-1, keepdims=True)
    xc = x - m
    v = jnp.mean(xc * xc, axis=-1, keepdims=True)
    return xc * jax.lax.rsqrt(v + EPS)


def _gelu(x):
    return jax.nn.gelu(x, approximate=True)


def _kernel(q_ref, k_ref, v_ref, sk_ref, ssmk_ref, dvec_ref, w1_ref, w2_ref, w3_ref, w4_ref,
            fw_ref, gi_ref, o_ref,
            kf_scr, xf_scr, yprev_scr, kext_scr, hb_scr, h_scr, xb_scr):
    s = pl.program_id(0)

    @pl.when(s == 0)
    def _init():
        fw = fw_ref[...]
        for i in range(NB):
            kf_scr[i] = jax.lax.dot_general(
                fw, ssmk_ref[:, i * C:(i + 1) * C],
                (((1,), (1,)), ((), ())), preferred_element_type=F32)
        yprev_scr[...] = jnp.zeros_like(yprev_scr)
        kext_scr[0:8, :] = jnp.zeros((8, D), F32)
        hb_scr[0:8, :] = jnp.zeros((8, D), F32)
        hb_scr[S + 8:S + 16, :] = jnp.zeros((8, D), F32)

    @pl.when(s < NT)
    def _phase1():
        slot = s % 2
        x = q_ref[...].astype(F32)
        qn = _ln(x)
        kext_scr[8:8 + T, :] = k_ref[...].astype(F32)
        sk = sk_ref[...].astype(F32)
        ksh = (kext_scr[8:8 + T, :] * sk[0:1, :] + kext_scr[7:7 + T, :] * sk[1:2, :]
               + kext_scr[6:6 + T, :] * sk[2:3, :] + kext_scr[5:5 + T, :] * sk[3:4, :])
        kext_scr[0:8, :] = kext_scr[T:T + 8, :]
        kv = ksh * v_ref[...].astype(F32)
        kvb = kv.astype(BF16)
        fw = fw_ref[...]
        ys = []
        for u in range(SUB):
            m = s * SUB + u
            xf_scr[m] = jnp.dot(fw, kvb[u * C:(u + 1) * C, :], preferred_element_type=F32)
            cols = []
            for lc in range(D // 128):
                lanes = slice(lc * 128, (lc + 1) * 128)
                halves = []
                for rh in range(2):
                    r0 = rh * 64

                    def body(j, acc, lanes=lanes, r0=r0, m=m):
                        ar, ai = acc
                        kr = kf_scr[m - j, r0:r0 + 64, lanes]
                        ki = kf_scr[m - j, C + r0:C + r0 + 64, lanes]
                        xr = xf_scr[j, r0:r0 + 64, lanes]
                        xi = xf_scr[j, C + r0:C + r0 + 64, lanes]
                        return (ar + kr * xr - ki * xi, ai + kr * xi + ki * xr)

                    z = jnp.zeros((64, 128), F32)
                    halves.append(jax.lax.fori_loop(0, m + 1, body, (z, z)))
                cols.append(halves)
            yf = jnp.concatenate(
                [jnp.concatenate([cols[lc][0][0] for lc in range(D // 128)], axis=1),
                 jnp.concatenate([cols[lc][1][0] for lc in range(D // 128)], axis=1),
                 jnp.concatenate([cols[lc][0][1] for lc in range(D // 128)], axis=1),
                 jnp.concatenate([cols[lc][1][1] for lc in range(D // 128)], axis=1)],
                axis=0).astype(BF16)
            y = (jnp.dot(gi_ref[0:C, :], yf, preferred_element_type=F32)
                 + jnp.dot(gi_ref[C:2 * C, :], yprev_scr[...], preferred_element_type=F32))
            yprev_scr[...] = yf
            ys.append(y)
        y = jnp.concatenate(ys, axis=0)
        y = y + kv * dvec_ref[...].astype(F32)
        h = x + qn * y
        xb = _ln(h)
        h_scr[slot] = h
        xb_scr[slot] = xb
        hb = _gelu(jnp.dot(_ln(xb).astype(BF16), w1_ref[...], preferred_element_type=F32))
        hb_scr[pl.ds(pl.multiple_of(8 + s * T, 8), T), :] = hb

    @pl.when(s > 0)
    def _phase2():
        p = s - 1
        slot = p % 2
        base = pl.multiple_of(p * T, 8)
        win = hb_scr[pl.ds(base, T + 16), :]
        lane = jax.lax.broadcasted_iota(jnp.int32, (T, D), 1)
        sh = jnp.where(lane < GRP, win[7:7 + T, :],
                       jnp.where(lane < 2 * GRP, win[9:9 + T, :],
                                 jnp.where(lane < 3 * GRP, win[6:6 + T, :], win[10:10 + T, :])))
        hs = jnp.dot(sh.astype(BF16), w2_ref[...], preferred_element_type=F32)
        x1 = xb_scr[slot] + hs
        a = _gelu(jnp.dot(_ln(x1).astype(BF16), w3_ref[...], preferred_element_type=F32))
        h2 = jnp.dot(a.astype(BF16), w4_ref[...], preferred_element_type=F32)
        o_ref[...] = (h_scr[slot] + x1 + h2).astype(o_ref.dtype)


@jax.jit
def pallas_sequential_preLN__ssm_conv_h3__mixer_s_mlp__prompt_kernel(
    A_q: jax.Array,
    A_k: jax.Array,
    A_v: jax.Array,
    A_shift_k: jax.Array,
    A_ssm_k: jax.Array,
    A_ssm_D: jax.Array,
    B_x: jax.Array,
    B_w1: jax.Array,
    B_w2: jax.Array,
    B_w3: jax.Array,
    B_w4: jax.Array,
):
    q = A_q.reshape(S, D)
    k = A_k.reshape(S, D)
    v = A_v.reshape(S, D)
    sk = A_shift_k.T
    dvec = A_ssm_D.reshape(1, D)
    fw_np, gi_np = _dft_constants()
    fw = jnp.asarray(fw_np, dtype=BF16)
    gi = jnp.asarray(gi_np, dtype=BF16)

    tile = pl.BlockSpec((T, D), lambda s: (jnp.minimum(s, NT - 1), 0))

    def full(shape):
        return pl.BlockSpec(shape, lambda s: (0,) * len(shape))

    out = pl.pallas_call(
        _kernel,
        grid=(NT + 1,),
        in_specs=[tile, tile, tile, full((4, D)), full((D, S)), full((1, D)),
                  full((D, D)), full((D, D)), full((D, FF)), full((FF, D)),
                  full((2 * C, C)), full((2 * C, 2 * C))],
        out_specs=pl.BlockSpec((T, D), lambda s: (jnp.maximum(s - 1, 0), 0)),
        out_shape=jax.ShapeDtypeStruct((S, D), A_q.dtype),
        scratch_shapes=[
            pltpu.VMEM((NB, 2 * C, D), F32),
            pltpu.VMEM((NB, 2 * C, D), F32),
            pltpu.VMEM((2 * C, D), BF16),
            pltpu.VMEM((T + 8, D), F32),
            pltpu.VMEM((S + 16, D), F32),
            pltpu.VMEM((2, T, D), F32),
            pltpu.VMEM((2, T, D), F32),
        ],
        compiler_params=pltpu.CompilerParams(
            dimension_semantics=("arbitrary",),
            vmem_limit_bytes=100 * 1024 * 1024,
        ),
    )(q, k, v, sk, A_ssm_k, dvec, B_w1, B_w2, B_w3, B_w4, fw, gi)
    return out.reshape(1, S, D)
```

```python
import numpy as np
import jax
import jax.numpy as jnp
import jax.experimental.pallas as pl
import jax.experimental.pallas.tpu as pltpu

S, D, FF = 2048, 640, 1728
C = 128
NB = S // C
T = 256
NT = S // T
SUB = T // C
GRP = D // 4
NG = 7
EPS = 1e-5
F32 = jnp.float32
BF16 = jnp.bfloat16


def _dft_constants():
    f = np.arange(C, dtype=np.float64)
    theta = np.pi * (2.0 * f + 1.0) / (2.0 * C)
    r = np.arange(C, dtype=np.float64)
    ang = theta[:, None] * r[None, :]
    fw = np.concatenate([np.cos(ang), -np.sin(ang)], axis=0)
    gi = np.concatenate([np.cos(ang.T), -np.sin(ang.T)], axis=1) / C
    return fw.astype(np.float32), gi.astype(np.float32)


def _group_table():
    pending = []
    tab = np.zeros((NT + 1, NG, 2), np.int32)
    tab[:, :, 0] = NB
    for st in range(1, NT - 1):
        for m in range(2 * st + 2, NB):
            pending.append((m, st))
        pending.sort()
        for g in range(NG):
            tab[st, g] = pending.pop(0)
    assert not pending
    return tab.reshape(-1)


def _ln(x):
    m = jnp.mean(x, axis=-1, keepdims=True)
    xc = x - m
    v = jnp.mean(xc * xc, axis=-1, keepdims=True)
    return xc * jax.lax.rsqrt(v + EPS)


def _gelu(x):
    return jax.nn.gelu(x, approximate=True)


def _cmul(k, x):
    kr, ki, xr, xi = k[0:C], k[C:2 * C], x[0:C], x[C:2 * C]
    return kr * xr - ki * xi, kr * xi + ki * xr


def _kernel(tab_ref, q_hbm, k_hbm, v_hbm, sk_hbm, ssmk_hbm, dvec_hbm, w1_hbm, w2_hbm, w3_hbm, w4_hbm,
            fw_hbm, gi_hbm, o_ref,
            q_v, k_v, v_v, sk_v, ssmk_v, dvec_v, w1_v, w2_v, w3_v, w4_v, fw_v, gi_v,
            kf_scr, xf_scr, yacc_scr, kext_scr, hb_scr, h_scr, xb_scr, a_scr, sem_tile, sem_misc):
    s = pl.program_id(0)

    def tile_copy(a, t):
        src, dst = ((q_hbm, q_v), (k_hbm, k_v), (v_hbm, v_v))[a]
        rows = pl.ds(pl.multiple_of(t * T, T), T)
        return pltpu.make_async_copy(src.at[rows], dst.at[rows], sem_tile.at[a, t])

    misc = ((fw_hbm, fw_v), (ssmk_hbm, ssmk_v), (sk_hbm, sk_v), (gi_hbm, gi_v), (dvec_hbm, dvec_v),
            (w1_hbm, w1_v), (w2_hbm, w2_v), (w3_hbm, w3_v), (w4_hbm, w4_v))

    def misc_copy(i):
        return pltpu.make_async_copy(misc[i][0], misc[i][1], sem_misc.at[i])

    @pl.when(s == 0)
    def _init():
        for i in range(2):
            misc_copy(i).start()
        kext_scr[0:8, :] = jnp.zeros((8, D), F32)
        hb_scr[0:8, :] = jnp.zeros((8, D), F32)
        hb_scr[S + 8:S + 16, :] = jnp.zeros((8, D), F32)
        yacc_scr[0] = jnp.zeros((2 * C, D), F32)
        yacc_scr[1] = jnp.zeros((2 * C, D), F32)
        yacc_scr[NB] = jnp.zeros((2 * C, D), F32)
        for i in range(2):
            misc_copy(i).wait()
        for a in (1, 2, 0):
            tile_copy(a, 0).start()
        for i in range(2, 6):
            misc_copy(i).start()
        for a in (1, 2, 0):
            tile_copy(a, 1).start()
        for i in range(6, 9):
            misc_copy(i).start()
        fw = fw_v[...]
        sgn = jnp.where(jax.lax.broadcasted_iota(jnp.int32, (C, D), 0) % 2 == 0, 1.0, -1.0).astype(F32)
        prev = None
        for i in range(NB):
            cur = jax.lax.dot_general(
                fw, ssmk_v[:, i * C:(i + 1) * C],
                (((1,), (1,)), ((), ())), preferred_element_type=F32)
            if prev is None:
                kf_scr[i] = cur
            else:
                kf_scr[i, 0:C] = cur[0:C] - sgn * prev[C:2 * C]
                kf_scr[i, C:2 * C] = cur[C:2 * C] + sgn * prev[0:C]
            prev = cur
        for i in range(2, 6):
            misc_copy(i).wait()
        for t in range(2, NT):
            for a in (1, 2, 0):
                tile_copy(a, t).start()

    @pl.when(s < NT)
    def _phase1():
        slot = s % 2
        for a in (1, 2, 0):
            tile_copy(a, s).wait()
        rows = pl.ds(pl.multiple_of(s * T, T), T)
        kext_scr[8:8 + T, :] = k_v[rows, :].astype(F32)
        sk = sk_v[...].astype(F32)
        ksh = (kext_scr[8:8 + T, :] * sk[0:1, :] + kext_scr[7:7 + T, :] * sk[1:2, :]
               + kext_scr[6:6 + T, :] * sk[2:3, :] + kext_scr[5:5 + T, :] * sk[3:4, :])
        kext_scr[0:8, :] = kext_scr[T:T + 8, :]
        kv = ksh * v_v[rows, :].astype(F32)
        kvb = kv.astype(BF16)
        fw = fw_v[...]
        xa = jnp.dot(fw, kvb[0:C, :], preferred_element_type=F32)
        xb_ = jnp.dot(fw, kvb[C:2 * C, :], preferred_element_type=F32)
        xf_scr[2 * s] = xa
        xf_scr[2 * s + 1] = xb_
        k0 = kf_scr[0]
        k1 = kf_scr[1]
        r0, i0 = _cmul(k0, xa)
        ya = yacc_scr[2 * s]
        za = jnp.concatenate([ya[0:C] + r0, ya[C:2 * C] + i0], axis=0).astype(BF16)
        r1, i1 = _cmul(k1, xa)
        r2, i2 = _cmul(k0, xb_)
        yb = yacc_scr[2 * s + 1]
        zb = jnp.concatenate([yb[0:C] + r1 + r2, yb[C:2 * C] + i1 + i2], axis=0).astype(BF16)
        gi = gi_v[...]
        y = jnp.concatenate([jnp.dot(gi, za, preferred_element_type=F32),
                             jnp.dot(gi, zb, preferred_element_type=F32)], axis=0)
        y = y + kv * dvec_v[...].astype(F32)
        x = q_v[rows, :].astype(F32)
        h = x + _ln(x) * y
        xb = _ln(h)
        h_scr[slot] = h
        xb_scr[slot] = xb
        hb = _gelu(jnp.dot(_ln(xb).astype(BF16), w1_v[...], preferred_element_type=F32))
        hb_scr[pl.ds(pl.multiple_of(8 + s * T, 8), T), :] = hb

    @pl.when(s == 0)
    def _hist0():
        xa = xf_scr[0]
        xb_ = xf_scr[1]
        for m in range(2, NB):
            r1, i1 = _cmul(kf_scr[m], xa)
            r2, i2 = _cmul(kf_scr[m - 1], xb_)
            yacc_scr[m, 0:C] = r1 + r2
            yacc_scr[m, C:2 * C] = i1 + i2
        for i in range(6, 9):
            misc_copy(i).wait()

    @pl.when(s > 0)
    def _phase2():
        p = s - 1
        slot = p % 2
        base = pl.multiple_of(p * T, 8)
        win = hb_scr[pl.ds(base, T + 16), :]
        lane = jax.lax.broadcasted_iota(jnp.int32, (T, D), 1)
        sh = jnp.where(lane < GRP, win[7:7 + T, :],
                       jnp.where(lane < 2 * GRP, win[9:9 + T, :],
                                 jnp.where(lane < 3 * GRP, win[6:6 + T, :], win[10:10 + T, :])))
        work = []
        for g in range(NG):
            m = tab_ref[(s * NG + g) * 2]
            t = tab_ref[(s * NG + g) * 2 + 1]
            for lc in range(D // 128):
                for rh in range(4):
                    work.append((m, t, lc, rh))

        def do_work(n):
            for _ in range(n):
                if not work:
                    return
                m, t, lc, rh = work.pop(0)
                ln_ = slice(lc * 128, (lc + 1) * 128)
                ra = slice(rh * 32, rh * 32 + 32)
                rb = slice(C + rh * 32, C + rh * 32 + 32)
                k1r, k1i = kf_scr[m - 2 * t, ra, ln_], kf_scr[m - 2 * t, rb, ln_]
                k2r, k2i = kf_scr[m - 2 * t - 1, ra, ln_], kf_scr[m - 2 * t - 1, rb, ln_]
                x1r, x1i = xf_scr[2 * t, ra, ln_], xf_scr[2 * t, rb, ln_]
                x2r, x2i = xf_scr[2 * t + 1, ra, ln_], xf_scr[2 * t + 1, rb, ln_]
                yacc_scr[m, ra, ln_] = (yacc_scr[m, ra, ln_] + (k1r * x1r - k1i * x1i)) + (k2r * x2r - k2i * x2i)
                yacc_scr[m, rb, ln_] = (yacc_scr[m, rb, ln_] + (k1r * x1i + k1i * x1r)) + (k2r * x2i + k2i * x2r)

        hs = jnp.dot(sh.astype(BF16), w2_v[...], preferred_element_type=F32)
        do_work(10)
        x1 = xb_scr[slot] + hs
        x1n = _ln(x1).astype(BF16)
        do_work(10)
        for c0 in range(0, FF, 256):
            c1 = min(c0 + 256, FF)
            a_scr[:, c0:c1] = _gelu(jax.lax.dot_general(
                x1n, w3_v[c0:c1, :], (((1,), (1,)), ((), ())), preferred_element_type=F32)).astype(BF16)
            do_work(10)
        for c0 in range(0, D, 128):
            h2 = jnp.dot(a_scr[...], w4_v[:, c0:c0 + 128], preferred_element_type=F32)
            o_ref[:, c0:c0 + 128] = (h_scr[slot, :, c0:c0 + 128] + x1[:, c0:c0 + 128] + h2).astype(o_ref.dtype)
            do_work(10)
        do_work(1000)


@jax.jit
def pallas_sequential_preLN__ssm_conv_h3__mixer_s_mlp__prompt_kernel(
    A_q: jax.Array,
    A_k: jax.Array,
    A_v: jax.Array,
    A_shift_k: jax.Array,
    A_ssm_k: jax.Array,
    A_ssm_D: jax.Array,
    B_x: jax.Array,
    B_w1: jax.Array,
    B_w2: jax.Array,
    B_w3: jax.Array,
    B_w4: jax.Array,
):
    q = A_q.reshape(S, D)
    k = A_k.reshape(S, D)
    v = A_v.reshape(S, D)
    sk = A_shift_k.T
    dvec = A_ssm_D.reshape(1, D)
    fw_np, gi_np = _dft_constants()
    fw = jnp.asarray(fw_np, dtype=BF16)
    gi = jnp.asarray(gi_np, dtype=BF16)
    tab = jnp.asarray(_group_table())

    hbm = pl.BlockSpec(memory_space=pltpu.HBM)
    grid_spec = pltpu.PrefetchScalarGridSpec(
        num_scalar_prefetch=1,
        grid=(NT + 1,),
        in_specs=[hbm] * 12,
        out_specs=pl.BlockSpec((T, D), lambda s, tab: (jnp.maximum(s - 1, 0), 0)),
        scratch_shapes=[
            pltpu.VMEM((S, D), BF16), pltpu.VMEM((S, D), BF16), pltpu.VMEM((S, D), BF16),
            pltpu.VMEM((4, D), BF16), pltpu.VMEM((D, S), BF16), pltpu.VMEM((1, D), BF16),
            pltpu.VMEM((D, D), BF16), pltpu.VMEM((D, D), BF16), pltpu.VMEM((FF, D), BF16),
            pltpu.VMEM((FF, D), BF16), pltpu.VMEM((2 * C, C), BF16), pltpu.VMEM((C, 2 * C), BF16),
            pltpu.VMEM((NB, 2 * C, D), F32),
            pltpu.VMEM((NB, 2 * C, D), F32),
            pltpu.VMEM((NB + 1, 2 * C, D), F32),
            pltpu.VMEM((T + 8, D), F32),
            pltpu.VMEM((S + 16, D), F32),
            pltpu.VMEM((2, T, D), F32),
            pltpu.VMEM((2, T, D), F32),
            pltpu.VMEM((T, FF), BF16),
            pltpu.SemaphoreType.DMA((3, NT)),
            pltpu.SemaphoreType.DMA((9,)),
        ],
    )
    out = pl.pallas_call(
        _kernel,
        grid_spec=grid_spec,
        out_shape=jax.ShapeDtypeStruct((S, D), A_q.dtype),
        compiler_params=pltpu.CompilerParams(
            dimension_semantics=("arbitrary",),
            vmem_limit_bytes=127 * 1024 * 1024,
        ),
    )(tab, q, k, v, sk, A_ssm_k, dvec, B_w1, B_w2, B_w3.T, B_w4, fw, gi)
    return out.reshape(1, S, D)
```

```python
import numpy as np
import jax
import jax.numpy as jnp
import jax.experimental.pallas as pl
import jax.experimental.pallas.tpu as pltpu

S, D, FF = 2048, 640, 1728
C = 128
NB = S // C
T = 256
NT = S // T
SUB = T // C
GRP = D // 4
NG = 7
EPS = 1e-5
F32 = jnp.float32
BF16 = jnp.bfloat16


def _dft_constants():
    f = np.arange(C, dtype=np.float64)
    theta = np.pi * (2.0 * f + 1.0) / (2.0 * C)
    r = np.arange(C, dtype=np.float64)
    ang = theta[:, None] * r[None, :]
    fw = np.concatenate([np.cos(ang), -np.sin(ang)], axis=0)
    gi = np.concatenate([np.cos(ang.T), -np.sin(ang.T)], axis=1) / C
    return fw.astype(np.float32), gi.astype(np.float32)


def _group_table():
    pending = []
    tab = np.zeros((NT + 1, NG, 2), np.int32)
    tab[:, :, 0] = NB
    for st in range(1, NT - 1):
        for m in range(2 * st + 2, NB):
            pending.append((m, st))
        pending.sort()
        for g in range(NG):
            tab[st, g] = pending.pop(0)
    assert not pending
    return tab.reshape(-1)


def _ln(x):
    m = jnp.mean(x, axis=-1, keepdims=True)
    xc = x - m
    v = jnp.mean(xc * xc, axis=-1, keepdims=True)
    return xc * jax.lax.rsqrt(v + EPS)


def _gelu(x):
    return jax.nn.gelu(x, approximate=True)


def _cmul(k, x):
    kr, ki, xr, xi = k[0:C], k[C:2 * C], x[0:C], x[C:2 * C]
    return kr * xr - ki * xi, kr * xi + ki * xr


def _kernel(tab_ref, q_hbm, k_hbm, v_hbm, sk_hbm, ssmk_hbm, dvec_hbm, w1_hbm, w2_hbm, w3_hbm, w4_hbm,
            fw_hbm, gi_hbm, o_ref,
            q_v, k_v, v_v, sk_v, ssmk_v, dvec_v, w1_v, w2_v, w3_v, w4_v, fw_v, gi_v,
            kf_scr, xf_scr, yacc_scr, kext_scr, hb_scr, h_scr, xb_scr, a_scr, sem_tile, sem_misc):
    s = pl.program_id(0)

    def tile_copy(a, t):
        src, dst = ((q_hbm, q_v), (k_hbm, k_v), (v_hbm, v_v))[a]
        rows = pl.ds(pl.multiple_of(t * T, T), T)
        return pltpu.make_async_copy(src.at[rows], dst.at[rows], sem_tile.at[a, t])

    misc = ((fw_hbm, fw_v), (ssmk_hbm, ssmk_v), (sk_hbm, sk_v), (gi_hbm, gi_v), (dvec_hbm, dvec_v),
            (w1_hbm, w1_v), (w2_hbm, w2_v), (w3_hbm, w3_v), (w4_hbm, w4_v))

    def misc_copy(i):
        return pltpu.make_async_copy(misc[i][0], misc[i][1], sem_misc.at[i])

    @pl.when(s == 0)
    def _init():
        for i in range(2):
            misc_copy(i).start()
        kext_scr[0:8, :] = jnp.zeros((8, D), F32)
        hb_scr[0:8, :] = jnp.zeros((8, D), F32)
        hb_scr[S + 8:S + 16, :] = jnp.zeros((8, D), F32)
        yacc_scr[0] = jnp.zeros((2 * C, D), F32)
        yacc_scr[1] = jnp.zeros((2 * C, D), F32)
        yacc_scr[NB] = jnp.zeros((2 * C, D), F32)
        for i in range(2):
            misc_copy(i).wait()
        for a in (1, 2, 0):
            tile_copy(a, 0).start()
        for i in range(2, 6):
            misc_copy(i).start()
        for a in (1, 2, 0):
            tile_copy(a, 1).start()
        for i in range(6, 9):
            misc_copy(i).start()
        fw = fw_v[...]
        sgn = jnp.where(jax.lax.broadcasted_iota(jnp.int32, (C, D), 0) % 2 == 0, 1.0, -1.0).astype(F32)
        prev = None
        for i in range(NB):
            cur = jax.lax.dot_general(
                fw, ssmk_v[:, i * C:(i + 1) * C],
                (((1,), (1,)), ((), ())), preferred_element_type=F32)
            if prev is None:
                kf_scr[i] = cur
            else:
                kf_scr[i, 0:C] = cur[0:C] - sgn * prev[C:2 * C]
                kf_scr[i, C:2 * C] = cur[C:2 * C] + sgn * prev[0:C]
            prev = cur
        for i in range(2, 6):
            misc_copy(i).wait()
        for t in range(2, NT):
            for a in (1, 2, 0):
                tile_copy(a, t).start()

    @pl.when(s < NT)
    def _phase1():
        slot = s % 2
        for a in (1, 2, 0):
            tile_copy(a, s).wait()
        rows = pl.ds(pl.multiple_of(s * T, T), T)
        kext_scr[8:8 + T, :] = k_v[rows, :].astype(F32)
        sk = sk_v[...].astype(F32)
        ksh = (kext_scr[8:8 + T, :] * sk[0:1, :] + kext_scr[7:7 + T, :] * sk[1:2, :]
               + kext_scr[6:6 + T, :] * sk[2:3, :] + kext_scr[5:5 + T, :] * sk[3:4, :])
        kext_scr[0:8, :] = kext_scr[T:T + 8, :]
        kv = ksh * v_v[rows, :].astype(F32)
        kvb = kv.astype(BF16)
        fw = fw_v[...]
        xa = jnp.dot(fw, kvb[0:C, :], preferred_element_type=F32)
        xb_ = jnp.dot(fw, kvb[C:2 * C, :], preferred_element_type=F32)
        xf_scr[2 * s] = xa
        xf_scr[2 * s + 1] = xb_
        k0 = kf_scr[0]
        k1 = kf_scr[1]
        r0, i0 = _cmul(k0, xa)
        ya = yacc_scr[2 * s]
        za = jnp.concatenate([ya[0:C] + r0, ya[C:2 * C] + i0], axis=0).astype(BF16)
        r1, i1 = _cmul(k1, xa)
        r2, i2 = _cmul(k0, xb_)
        yb = yacc_scr[2 * s + 1]
        zb = jnp.concatenate([yb[0:C] + r1 + r2, yb[C:2 * C] + i1 + i2], axis=0).astype(BF16)
        gi = gi_v[...]
        y = jnp.concatenate([jnp.dot(gi, za, preferred_element_type=F32),
                             jnp.dot(gi, zb, preferred_element_type=F32)], axis=0)
        y = y + kv * dvec_v[...].astype(F32)
        x = q_v[rows, :].astype(F32)
        h = x + _ln(x) * y
        xb = _ln(h)
        h_scr[slot] = h
        xb_scr[slot] = xb
        hb = _gelu(jnp.dot(_ln(xb).astype(BF16), w1_v[...], preferred_element_type=F32))
        hb_scr[pl.ds(pl.multiple_of(8 + s * T, 8), T), :] = hb

    @pl.when(s == 0)
    def _hist0():
        xa = xf_scr[0]
        xb_ = xf_scr[1]
        for m in range(2, NB):
            r1, i1 = _cmul(kf_scr[m], xa)
            r2, i2 = _cmul(kf_scr[m - 1], xb_)
            yacc_scr[m, 0:C] = r1 + r2
            yacc_scr[m, C:2 * C] = i1 + i2
        for i in range(6, 9):
            misc_copy(i).wait()

    def _phase2(with_groups):
        p = s - 1
        slot = p % 2
        base = pl.multiple_of(p * T, 8)
        win = hb_scr[pl.ds(base, T + 16), :]
        lane = jax.lax.broadcasted_iota(jnp.int32, (T, D), 1)
        sh = jnp.where(lane < GRP, win[7:7 + T, :],
                       jnp.where(lane < 2 * GRP, win[9:9 + T, :],
                                 jnp.where(lane < 3 * GRP, win[6:6 + T, :], win[10:10 + T, :])))
        work = []
        for g in range(NG if with_groups else 0):
            m = tab_ref[(s * NG + g) * 2]
            t = tab_ref[(s * NG + g) * 2 + 1]
            for lc in range(D // 128):
                for rh in range(4):
                    work.append((m, t, lc, rh))

        def do_work(n):
            for _ in range(n):
                if not work:
                    return
                m, t, lc, rh = work.pop(0)
                ln_ = slice(lc * 128, (lc + 1) * 128)
                ra = slice(rh * 32, rh * 32 + 32)
                rb = slice(C + rh * 32, C + rh * 32 + 32)
                k1r, k1i = kf_scr[m - 2 * t, ra, ln_], kf_scr[m - 2 * t, rb, ln_]
                k2r, k2i = kf_scr[m - 2 * t - 1, ra, ln_], kf_scr[m - 2 * t - 1, rb, ln_]
                x1r, x1i = xf_scr[2 * t, ra, ln_], xf_scr[2 * t, rb, ln_]
                x2r, x2i = xf_scr[2 * t + 1, ra, ln_], xf_scr[2 * t + 1, rb, ln_]
                yacc_scr[m, ra, ln_] = (yacc_scr[m, ra, ln_] + (k1r * x1r - k1i * x1i)) + (k2r * x2r - k2i * x2i)
                yacc_scr[m, rb, ln_] = (yacc_scr[m, rb, ln_] + (k1r * x1i + k1i * x1r)) + (k2r * x2i + k2i * x2r)

        hs = jnp.dot(sh.astype(BF16), w2_v[...], preferred_element_type=F32)
        do_work(4)
        x1 = xb_scr[slot] + hs
        x1n = _ln(x1).astype(BF16)
        do_work(4)
        for c0 in range(0, FF, 256):
            c1 = min(c0 + 256, FF)
            a_scr[:, c0:c1] = _gelu(jax.lax.dot_general(
                x1n, w3_v[c0:c1, :], (((1,), (1,)), ((), ())), preferred_element_type=F32)).astype(BF16)
            do_work(8)
        for c0 in range(0, D, 128):
            h2 = jnp.dot(a_scr[...], w4_v[:, c0:c0 + 128], preferred_element_type=F32)
            o_ref[:, c0:c0 + 128] = (h_scr[slot, :, c0:c0 + 128] + x1[:, c0:c0 + 128] + h2).astype(o_ref.dtype)
            do_work(16)
        do_work(1000)

    @pl.when(jnp.logical_and(s > 0, s < NT - 1))
    def _p2a():
        _phase2(True)

    @pl.when(s >= NT - 1)
    def _p2b():
        _phase2(False)


@jax.jit
def pallas_sequential_preLN__ssm_conv_h3__mixer_s_mlp__prompt_kernel(
    A_q: jax.Array,
    A_k: jax.Array,
    A_v: jax.Array,
    A_shift_k: jax.Array,
    A_ssm_k: jax.Array,
    A_ssm_D: jax.Array,
    B_x: jax.Array,
    B_w1: jax.Array,
    B_w2: jax.Array,
    B_w3: jax.Array,
    B_w4: jax.Array,
):
    q = A_q.reshape(S, D)
    k = A_k.reshape(S, D)
    v = A_v.reshape(S, D)
    sk = A_shift_k.T
    dvec = A_ssm_D.reshape(1, D)
    fw_np, gi_np = _dft_constants()
    fw = jnp.asarray(fw_np, dtype=BF16)
    gi = jnp.asarray(gi_np, dtype=BF16)
    tab = jnp.asarray(_group_table())

    hbm = pl.BlockSpec(memory_space=pltpu.HBM)
    grid_spec = pltpu.PrefetchScalarGridSpec(
        num_scalar_prefetch=1,
        grid=(NT + 1,),
        in_specs=[hbm] * 12,
        out_specs=pl.BlockSpec((T, D), lambda s, tab: (jnp.maximum(s - 1, 0), 0)),
        scratch_shapes=[
            pltpu.VMEM((S, D), BF16), pltpu.VMEM((S, D), BF16), pltpu.VMEM((S, D), BF16),
            pltpu.VMEM((4, D), BF16), pltpu.VMEM((D, S), BF16), pltpu.VMEM((1, D), BF16),
            pltpu.VMEM((D, D), BF16), pltpu.VMEM((D, D), BF16), pltpu.VMEM((FF, D), BF16),
            pltpu.VMEM((FF, D), BF16), pltpu.VMEM((2 * C, C), BF16), pltpu.VMEM((C, 2 * C), BF16),
            pltpu.VMEM((NB, 2 * C, D), F32),
            pltpu.VMEM((NB, 2 * C, D), F32),
            pltpu.VMEM((NB + 1, 2 * C, D), F32),
            pltpu.VMEM((T + 8, D), F32),
            pltpu.VMEM((S + 16, D), F32),
            pltpu.VMEM((2, T, D), F32),
            pltpu.VMEM((2, T, D), F32),
            pltpu.VMEM((T, FF), BF16),
            pltpu.SemaphoreType.DMA((3, NT)),
            pltpu.SemaphoreType.DMA((9,)),
        ],
    )
    out = pl.pallas_call(
        _kernel,
        grid_spec=grid_spec,
        out_shape=jax.ShapeDtypeStruct((S, D), A_q.dtype),
        compiler_params=pltpu.CompilerParams(
            dimension_semantics=("arbitrary",),
            vmem_limit_bytes=127 * 1024 * 1024,
        ),
    )(tab, q, k, v, sk, A_ssm_k, dvec, B_w1, B_w2, B_w3.T, B_w4, fw, gi)
    return out.reshape(1, S, D)
```
